```python
import jax
import jax.numpy as jnp

def _softmax(x, axis=-1):
    return jax.nn.softmax(x, axis=axis)

def _gelu(x):
    return jax.nn.gelu(x, approximate=True)

def _silu(x):
    return jax.nn.silu(x)

def _sigmoid(x):
    return jax.nn.sigmoid(x)

def _layernorm(x, axis=-1, eps=1e-05):
    m = jnp.mean(x, axis=axis, keepdims=True)
    v = jnp.var(x, axis=axis, keepdims=True)
    return (x - m) / jnp.sqrt(v + eps)

def _scatter_add(tgt, idx, src, axis=0):
    return tgt.at[idx].add(src)

def _segment_sum(src, seg, n):
    return jax.ops.segment_sum(src, seg, n)

class _Rng:

    def __init__(self, key):
        self._k = key

    def _next(self):
        self._k, sub = jax.random.split(self._k)
        return sub

    def normal(self, shape):
        return jax.random.normal(self._next(), shape, dtype=jnp.bfloat16)

    def randint(self, lo, hi, shape):
        return jax.random.randint(self._next(), shape, lo, hi, dtype=jnp.int32)

    def uniform(self, shape, lo=0.0, hi=1.0):
        return jax.random.uniform(self._next(), shape, jnp.bfloat16, lo, hi)

    def permutation(self, n):
        return jax.random.permutation(self._next(), n)
kernel_name = 'standalone__dilated_atrous__vision'

def setup_inputs():
    _rng = _Rng(jax.random.key(int.from_bytes(__import__("os").urandom(4), "little")))
    _w = lambda a: (lambda t: t.astype(jnp.bfloat16) if jnp.issubdtype(t.dtype, jnp.floating) else t)(jnp.asarray(a))
    H = W = 384
    C = 384
    k = 1
    return {'x': _w((lambda *s: _rng.normal(s) * 0.05)(1, H, W, C)), 'w': _w((lambda *s: _rng.normal(s) * 0.05)(k, k, C, C) * (1.0 / (k * C ** 0.5)))}

def reference(x, w):
    B, H, W, C = x.shape
    k = 1
    rate = 2
    pad = (k - 1) * rate // 2
    xp = jnp.pad(x, ((0, 0), (pad, pad), (pad, pad), (0, 0)))
    out = jnp.zeros_like(x)
    for i in range(k):
        for j in range(k):
            tap = xp[:, i * rate:i * rate + H, j * rate:j * rate + W, :].copy()
            out = out + jnp.einsum('bhwc,co->bhwo', tap, w[i, j])
    return out
```

```python
import jax
import jax.numpy as jnp
from jax import lax
import jax.experimental.pallas as pl
import jax.experimental.pallas.tpu as pltpu

_S = 6
_TG = 192
_TR = 32
_SH = 1
_TW = 48
_SUB = 96
_G0 = 4
_TAIL = 2
_M0 = 2


def _kernel(x_hbm, w_hbm, o_hbm, buf_a, buf_b, w_buf, rsem, osem, wsem):
    S, tg, tr, sh, tw, sub = _S, _TG, _TR, _SH, _TW, _SUB
    C = x_hbm.shape[-1]
    n = x_hbm.shape[1] // tg
    npairs = n // 2
    nc = tg // tr
    ns = S * tg // sub
    R = ns // nc
    K = (n - _G0) // (2 * R)

    def in_slot(pair, u):
        if u % 2 == 0:
            return buf_a.at[pair + u // 2]
        return buf_b.at[pair + (u + 1) // 2]

    def aligned(v, m):
        return v if isinstance(v, int) else pl.multiple_of(v, m)

    def request(pair, c, last=None):
        u, i = divmod(c, nc)
        g = 2 * pair + u
        rows = pl.ds(aligned(g * tg + i * tr, tr), tr)
        dst = in_slot(pair, u)
        if last is not None and u == 2 * R - 1 and i >= nc - _TAIL:
            g = jnp.where(last, n, g)
        for lo, hi, priority in ((0, sh, 0), (sh, S, 1)):
            pltpu.make_async_copy(
                x_hbm.at[lo:hi, rows, :],
                dst.at[lo:hi, pl.ds(i * tr, tr), :],
                rsem.at[g],
            ).start(priority=priority)

    def wait_read(pair, u):
        slot = in_slot(pair, u)
        pltpu.make_async_copy(slot, slot, rsem.at[2 * pair + u]).wait()

    def write_pair(m):
        for u, buf in ((0, buf_b), (1, buf_a)):
            for r in range(0, tg, tw):
                rows = pl.ds(aligned((2 * m + u) * tg + r, tw), tw)
                pltpu.make_async_copy(
                    buf.at[m, :, pl.ds(r, tw), :], o_hbm.at[:, rows, :], osem
                ).start()

    def matmul(x):
        y = jnp.dot(x, w_buf[...], preferred_element_type=jnp.float32)
        return y.astype(o_hbm.dtype)

    w_copy = pltpu.make_async_copy(w_hbm, w_buf, wsem)
    for c in range(_G0 * nc):
        request(0, c)
        if c == 2:
            w_copy.start()
        if c >= 2:
            pl.delay(150)
    w_copy.wait()

    def read_phase(k, carry):
        pair = _G0 // 2 + R * k
        for half in range(2):
            src, dst = (
                (buf_a.at[k], buf_b.at[k]) if half == 0
                else (buf_b.at[k + 1], buf_a.at[k])
            )
            for u in range(R):
                wait_read(pair, half * R - _G0 + u)
            c = half * ns
            for s in range(S):
                for r in range(0, tg, sub):
                    request(pair, c, k == K - 1)
                    dst[s, pl.ds(r, sub), :] = matmul(src[s, pl.ds(r, sub), :])
                    c += 1
        return carry

    lax.fori_loop(0, K, read_phase, 0)

    for g in range(n - _G0, n - 1):
        wait_read(0, g)
    last = in_slot(0, n - 1)
    head = last.at[:, pl.ds(0, (nc - _TAIL) * tr), :]
    tail = last.at[:, pl.ds((nc - _TAIL) * tr, _TAIL * tr), :]
    pltpu.make_async_copy(head, head, rsem.at[n - 1]).wait()
    for m in range(_M0):
        write_pair(m)
    pltpu.make_async_copy(tail, tail, rsem.at[n]).wait()

    def granule(src, dst):
        dst[...] = matmul(src[...].reshape(S * tg, C)).reshape(S, tg, -1)

    def write_phase(k, m):
        granule(buf_a.at[k], buf_b.at[k])
        pl.when(m < k)(lambda: write_pair(m))
        m = jnp.where(m < k, m + 1, m)
        granule(buf_b.at[k + 1], buf_a.at[k])
        write_pair(m)
        return m + 1

    lax.fori_loop(K, npairs, write_phase, jnp.int32(_M0))
    pltpu.make_async_copy(o_hbm, o_hbm, osem).wait()


@jax.jit
def pallas_standalone__dilated_atrous__vision_kernel(x: jax.Array, w: jax.Array):
    B, H, W, C = x.shape
    O = w.shape[-1]
    L = B * H * W // _S
    npairs = L // _TG // 2
    out = pl.pallas_call(
        _kernel,
        in_specs=[pl.BlockSpec(memory_space=pl.ANY)] * 2,
        out_specs=pl.BlockSpec(memory_space=pl.ANY),
        out_shape=jax.ShapeDtypeStruct((_S, L, O), x.dtype),
        scratch_shapes=[
            pltpu.VMEM((npairs, _S, _TG, C), x.dtype),
            pltpu.VMEM((npairs + 1, _S, _TG, C), x.dtype),
            pltpu.VMEM((C, O), w.dtype),
            pltpu.SemaphoreType.DMA((2 * npairs + 1,)),
            pltpu.SemaphoreType.DMA(()),
            pltpu.SemaphoreType.DMA(()),
        ],
        compiler_params=pltpu.CompilerParams(vmem_limit_bytes=125 * 1024 * 1024),
    )(x.reshape(_S, L, C), w.reshape(C, O))
    return out.reshape(B, H, W, O)
```

```python
import jax
import jax.numpy as jnp
from jax import lax
import jax.experimental.pallas as pl
import jax.experimental.pallas.tpu as pltpu

_S = 6
_TG = 192
_TR = 32
_SH = 1
_TW = 48
_SUB = 96
_G0 = 8
_TAIL = 4
_M0 = 2


def _kernel(x_hbm, w_hbm, o_hbm, buf_a, buf_b, w_buf, rsem, osem, wsem):
    C = x_hbm.shape[-1]
    n = x_hbm.shape[1] // _TG
    nc = _TG // _TR
    ns = _S * _TG // _SUB
    R = ns // nc
    K = (n - _G0) // (2 * R)
    assert ns == R * nc and n == _G0 + 2 * R * K and _G0 % 2 == 0 and _M0 <= K

    def aligned(v, m):
        return v if isinstance(v, int) else pl.multiple_of(v, m)

    def in_slot(pair, u):
        if u % 2 == 0:
            return buf_a.at[pair + u // 2]
        return buf_b.at[pair + (u + 1) // 2]

    def request(pair, c, last=None):
        u, i = divmod(c, nc)
        g = 2 * pair + u
        rows = pl.ds(aligned(g * _TG + i * _TR, _TR), _TR)
        dst = in_slot(pair, u)
        if last is not None and u == 2 * R - 1 and i >= nc - _TAIL:
            g = jnp.where(last, n, g)
        for lo, hi, priority in ((0, _SH, 0), (_SH, _S, 1)):
            pltpu.make_async_copy(
                x_hbm.at[lo:hi, rows, :],
                dst.at[lo:hi, pl.ds(i * _TR, _TR), :],
                rsem.at[g],
            ).start(priority=priority)

    def wait_filled(ref, sem):
        pltpu.make_async_copy(ref, ref, sem).wait()

    def write_pair(m):
        for u, buf in ((0, buf_b), (1, buf_a)):
            for r in range(0, _TG, _TW):
                rows = pl.ds(aligned((2 * m + u) * _TG + r, _TW), _TW)
                pltpu.make_async_copy(
                    buf.at[m, :, pl.ds(r, _TW), :], o_hbm.at[:, rows, :], osem
                ).start()

    def matmul(x):
        y = jnp.dot(x, w_buf[...], preferred_element_type=jnp.float32)
        return y.astype(o_hbm.dtype)

    w_copy = pltpu.make_async_copy(w_hbm, w_buf, wsem)
    for c in range(_G0 * nc):
        request(0, c)
        if c == 2:
            w_copy.start()
    w_copy.wait()

    def read_phase(k, carry):
        pair = _G0 // 2 + R * k
        for half, (src, dst) in enumerate(
            ((buf_a.at[k], buf_b.at[k]), (buf_b.at[k + 1], buf_a.at[k]))
        ):
            for u in range(half * R - _G0, (half + 1) * R - _G0):
                wait_filled(in_slot(pair, u), rsem.at[2 * pair + u])
            c = half * ns
            for s in range(_S):
                for r in range(0, _TG, _SUB):
                    request(pair, c, k == K - 1)
                    dst[s, pl.ds(r, _SUB), :] = matmul(src[s, pl.ds(r, _SUB), :])
                    c += 1
        return carry

    lax.fori_loop(0, K, read_phase, 0)

    for g in range(n - _G0, n - 1):
        wait_filled(in_slot(0, g), rsem.at[g])
    split = (nc - _TAIL) * _TR
    wait_filled(in_slot(0, n - 1).at[:, pl.ds(0, split), :], rsem.at[n - 1])
    for m in range(_M0):
        write_pair(m)
    wait_filled(in_slot(0, n - 1).at[:, pl.ds(split, _TG - split), :], rsem.at[n])

    def granule(src, dst):
        dst[...] = matmul(src[...].reshape(_S * _TG, C)).reshape(dst.shape)

    def write_phase(k, m):
        granule(buf_a.at[k], buf_b.at[k])
        pl.when(m < k)(lambda: write_pair(m))
        m = jnp.where(m < k, m + 1, m)
        granule(buf_b.at[k + 1], buf_a.at[k])
        write_pair(m)
        return m + 1

    assert _M0 + 2 * (n // 2 - K) >= n // 2
    lax.fori_loop(K, n // 2, write_phase, jnp.int32(_M0))
    wait_filled(o_hbm, osem)


@jax.jit
def pallas_standalone__dilated_atrous__vision_kernel(x: jax.Array, w: jax.Array):
    B, H, W, C = x.shape
    assert w.shape == (1, 1, C, C) and (B * H * W) % (2 * _S * _TG) == 0
    L = B * H * W // _S
    npairs = L // (2 * _TG)
    out = pl.pallas_call(
        _kernel,
        in_specs=[pl.BlockSpec(memory_space=pl.ANY)] * 2,
        out_specs=pl.BlockSpec(memory_space=pl.ANY),
        out_shape=jax.ShapeDtypeStruct((_S, L, C), x.dtype),
        scratch_shapes=[
            pltpu.VMEM((npairs, _S, _TG, C), x.dtype),
            pltpu.VMEM((npairs + 1, _S, _TG, C), x.dtype),
            pltpu.VMEM((C, C), w.dtype),
            pltpu.SemaphoreType.DMA((2 * npairs + 1,)),
            pltpu.SemaphoreType.DMA(()),
            pltpu.SemaphoreType.DMA(()),
        ],
        compiler_params=pltpu.CompilerParams(vmem_limit_bytes=118 * 1024 * 1024),
    )(x.reshape(_S, L, C), w.reshape(C, C))
    return out.reshape(B, H, W, C)
```
